```python
import os as _os
_os.environ.setdefault("JAX_PLATFORMS", "cpu")
import jax
import jax.numpy as jnp

def _softmax(x, axis=-1):
    return jax.nn.softmax(x, axis=axis)
def _gelu(x):
    return jax.nn.gelu(x, approximate=True)
def _silu(x):
    return jax.nn.silu(x)
def _sigmoid(x):
    return jax.nn.sigmoid(x)
def _layernorm(x, axis=-1, eps=1e-5):
    m = jnp.mean(x, axis=axis, keepdims=True)
    v = jnp.var(x, axis=axis, keepdims=True)
    return (x - m) / jnp.sqrt(v + eps)
def _scatter_add(tgt, idx, src, axis=0):
    return tgt.at[idx].add(src)
def _segment_sum(src, seg, n):
    return jax.ops.segment_sum(src, seg, n)
class _Rng:
    def __init__(self, key):
        self._k = key
    def _next(self):
        self._k, sub = jax.random.split(self._k)
        return sub
    def normal(self, shape):
        return jax.random.normal(self._next(), shape, dtype=jnp.bfloat16)
    def randint(self, lo, hi, shape):
        return jax.random.randint(self._next(), shape, lo, hi, dtype=jnp.int32)
    def uniform(self, shape, lo=0.0, hi=1.0):
        return jax.random.uniform(self._next(), shape, jnp.bfloat16, lo, hi)
    def permutation(self, n):
        return jax.random.permutation(self._next(), n)


kernel_name = 'standalone__instancenorm__sampling'

def setup_inputs():
    _rng = _Rng(jax.random.key(int.from_bytes(__import__("os").urandom(4), "little")))
    _w = (lambda a: (lambda t: t.astype(jnp.bfloat16) if jnp.issubdtype(t.dtype, jnp.floating) else t)(jnp.asarray(a)))
    B, C, H, W = 16, 640, 16, 32
    return {
        "x": _w((lambda *s: _rng.normal(s) * 0.05)(B, C, H, W)),
        "g": _w((lambda *s: _rng.normal(s) * 0.05)(C) + 1.0),
        "b": _w((lambda *s: _rng.normal(s) * 0.05)(C)),
    }

def reference(x, g, b):
    mu = x.mean(axis=(-2, -1), keepdims=True)
    var = ((x - mu) * (x - mu)).mean(axis=(-2, -1), keepdims=True)
    xhat = (x - mu) / jnp.sqrt(var + 1e-5)
    return xhat * g.reshape(1, -1, 1, 1) + b.reshape(1, -1, 1, 1)
```

```python
import jax
import jax.numpy as jnp
from jax import lax
import jax.experimental.pallas as pl
import jax.experimental.pallas.tpu as pltpu

_EPS = 1e-5
_LANES = 128
_READ_WINDOW = 2


def _normalize(x_ref, o_ref, gamma, beta):
    inv_n = 1.0 / x_ref.shape[0]
    xf = x_ref[...].astype(jnp.float32)
    mu = jnp.sum(xf, axis=0, keepdims=True) * inv_n
    d = xf - mu
    var = jnp.sum(d * d, axis=0, keepdims=True) * inv_n
    scale = lax.rsqrt(var + _EPS) * gamma
    o_ref[...] = (d * scale + beta).astype(o_ref.dtype)


@jax.jit
def pallas_standalone__instancenorm__sampling_kernel(
    x: jax.Array,
    g: jax.Array,
    b: jax.Array,
):
    B, C, H, W = x.shape
    N = H * W
    CT = C // _LANES
    K = _READ_WINDOW
    first = B - 1

    def kernel_function(x_hbm, g_hbm, b_hbm, o_hbm,
                        xbuf, obuf, gbuf, bbuf, rsem, wsem, gsem):
        def read(i):
            return pltpu.make_async_copy(x_hbm.at[i], xbuf.at[i], rsem.at[i])

        copy_g = pltpu.make_async_copy(g_hbm, gbuf, gsem.at[0])
        copy_b = pltpu.make_async_copy(b_hbm, bbuf, gsem.at[1])
        read(0).start()
        copy_g.start()
        copy_b.start()
        for i in range(1, K):
            read(i).start()
        copy_g.wait()
        copy_b.wait()
        gv = gbuf[...].astype(jnp.float32)
        bv = bbuf[...].astype(jnp.float32)
        gamma = jnp.concatenate([gv[i:i + 1] for i in range(CT)], axis=1)
        beta = jnp.concatenate([bv[i:i + 1] for i in range(CT)], axis=1)

        def body(i, carry):
            read(i).wait()

            @pl.when(i + K < B)
            def _():
                read(i + K).start()

            _normalize(xbuf.at[i], obuf.at[i], gamma, beta)
            return carry

        lax.fori_loop(0, first, body, None)

        bulk = pltpu.make_async_copy(
            obuf.at[pl.ds(0, first)], o_hbm.at[pl.ds(0, first)], wsem.at[0])
        bulk.start()
        tail = []
        for i in range(first, B):
            read(i).wait()
            _normalize(xbuf.at[i], obuf.at[i], gamma, beta)
            w = pltpu.make_async_copy(
                obuf.at[i], o_hbm.at[i], wsem.at[1 + i - first])
            w.start()
            tail.append(w)
        bulk.wait()
        for w in tail:
            w.wait()

    xt = x.transpose(0, 2, 3, 1).reshape(B, N, C)
    y = pl.pallas_call(
        kernel_function,
        in_specs=[pl.BlockSpec(memory_space=pl.ANY)] * 3,
        out_specs=pl.BlockSpec(memory_space=pl.ANY),
        out_shape=jax.ShapeDtypeStruct((B, N, C), x.dtype),
        scratch_shapes=[
            pltpu.VMEM((B, N, C), x.dtype),
            pltpu.VMEM((B, N, C), x.dtype),
            pltpu.VMEM((CT, _LANES), g.dtype),
            pltpu.VMEM((CT, _LANES), b.dtype),
            pltpu.SemaphoreType.DMA((B,)),
            pltpu.SemaphoreType.DMA((1 + B - first,)),
            pltpu.SemaphoreType.DMA((2,)),
        ],
        compiler_params=pltpu.CompilerParams(vmem_limit_bytes=40 * 1024 * 1024),
    )(xt, g.reshape(CT, _LANES), b.reshape(CT, _LANES))
    return y.reshape(B, H, W, C).transpose(0, 3, 1, 2)
```

```python
import jax
import jax.numpy as jnp
from jax import lax
import jax.experimental.pallas as pl
import jax.experimental.pallas.tpu as pltpu

_EPS = 1e-5
_LANES = 128


def _normalize(x_ref, o_ref, gamma, beta):
    inv_n = 1.0 / x_ref.shape[0]
    xf = x_ref[...].astype(jnp.float32)
    mu = jnp.sum(xf, axis=0, keepdims=True) * inv_n
    d = xf - mu
    var = jnp.sum(d * d, axis=0, keepdims=True) * inv_n
    scale = lax.rsqrt(var + _EPS) * gamma
    o_ref[...] = (d * scale + beta).astype(o_ref.dtype)


@jax.jit
def pallas_standalone__instancenorm__sampling_kernel(
    x: jax.Array,
    g: jax.Array,
    b: jax.Array,
):
    B, C, H, W = x.shape
    N = H * W
    CT = C // _LANES
    n_read = (5 * B) // 8
    n_write = B // 2

    def kernel_function(x_hbm, g_hbm, b_hbm, o_hbm,
                        xbuf, obuf, gbuf, bbuf, rsem, wsem, psem):
        def copy(src, dst, lo, hi, sem):
            rows = pl.ds(lo, hi - lo)
            return pltpu.make_async_copy(src.at[rows], dst.at[rows], sem)

        read_a = copy(x_hbm, xbuf, 0, n_read, rsem.at[0])
        read_b = copy(x_hbm, xbuf, n_read, B, rsem.at[1])
        write_a = copy(obuf, o_hbm, 0, n_write, wsem.at[0])
        write_b = copy(obuf, o_hbm, n_write, B, wsem.at[1])
        copy_g = pltpu.make_async_copy(g_hbm, gbuf, psem.at[0])
        copy_b = pltpu.make_async_copy(b_hbm, bbuf, psem.at[1])

        read_a.start(priority=1)
        read_b.start(priority=1)
        copy_g.start()
        copy_b.start()
        copy_g.wait()
        copy_b.wait()
        gv = gbuf[...].astype(jnp.float32)
        bv = bbuf[...].astype(jnp.float32)
        gamma = jnp.concatenate([gv[i:i + 1] for i in range(CT)], axis=1)
        beta = jnp.concatenate([bv[i:i + 1] for i in range(CT)], axis=1)

        def normalize_sample(i, carry):
            _normalize(xbuf.at[i], obuf.at[i], gamma, beta)
            return carry

        read_a.wait()
        lax.fori_loop(0, n_write, normalize_sample, None)
        write_a.start()
        lax.fori_loop(n_write, n_read, normalize_sample, None)
        read_b.wait()
        lax.fori_loop(n_read, B, normalize_sample, None)
        write_b.start()
        write_a.wait()
        write_b.wait()

    xt = x.transpose(0, 2, 3, 1).reshape(B, N, C)
    y = pl.pallas_call(
        kernel_function,
        in_specs=[pl.BlockSpec(memory_space=pl.ANY)] * 3,
        out_specs=pl.BlockSpec(memory_space=pl.ANY),
        out_shape=jax.ShapeDtypeStruct((B, N, C), x.dtype),
        scratch_shapes=[
            pltpu.VMEM((B, N, C), x.dtype),
            pltpu.VMEM((B, N, C), x.dtype),
            pltpu.VMEM((CT, _LANES), g.dtype),
            pltpu.VMEM((CT, _LANES), b.dtype),
            pltpu.SemaphoreType.DMA((2,)),
            pltpu.SemaphoreType.DMA((2,)),
            pltpu.SemaphoreType.DMA((2,)),
        ],
        compiler_params=pltpu.CompilerParams(vmem_limit_bytes=40 * 1024 * 1024),
    )(xt, g.reshape(CT, _LANES), b.reshape(CT, _LANES))
    return y.reshape(B, H, W, C).transpose(0, 3, 1, 2)
```

```python
import jax
import jax.numpy as jnp
from jax import lax
import jax.experimental.pallas as pl
import jax.experimental.pallas.tpu as pltpu

_EPS = 1e-5
_LANES = 128
_GROUP = 4
_PIECE = 32


def _normalize(x_ref, o_ref, gamma, beta):
    inv_n = 1.0 / x_ref.shape[0]
    xf = x_ref[...].astype(jnp.float32)
    mu = jnp.sum(xf, axis=0, keepdims=True) * inv_n
    d = xf - mu
    var = jnp.sum(d * d, axis=0, keepdims=True) * inv_n
    scale = lax.rsqrt(var + _EPS) * gamma
    o_ref[...] = (d * scale + beta).astype(o_ref.dtype)


@jax.jit
def pallas_standalone__instancenorm__sampling_kernel(
    x: jax.Array,
    g: jax.Array,
    b: jax.Array,
):
    B, C, H, W = x.shape
    N = H * W
    R = B * N
    CT = C // _LANES
    n_read = (5 * B) // 8

    def kernel_function(x_hbm, g_hbm, b_hbm, o_hbm,
                        xbuf, obuf, gbuf, bbuf, rsem, wsem, psem):
        def copy(src, dst, start, rows, sem):
            return pltpu.make_async_copy(
                src.at[pl.ds(start, rows)], dst.at[pl.ds(start, rows)], sem)

        read_a = copy(x_hbm, xbuf, 0, n_read * N, rsem.at[0])
        read_b = copy(x_hbm, xbuf, n_read * N, R - n_read * N, rsem.at[1])
        copy_g = pltpu.make_async_copy(g_hbm, gbuf, psem.at[0])
        copy_b = pltpu.make_async_copy(b_hbm, bbuf, psem.at[1])

        read_a.start(priority=1)
        read_b.start(priority=1)
        copy_g.start()
        copy_b.start()
        copy_g.wait()
        copy_b.wait()
        gv = gbuf[...].astype(jnp.float32)
        bv = bbuf[...].astype(jnp.float32)
        gamma = jnp.concatenate([gv[i:i + 1] for i in range(CT)], axis=1)
        beta = jnp.concatenate([bv[i:i + 1] for i in range(CT)], axis=1)

        def normalize(lo, hi):
            def body(i, carry):
                rows = pl.ds(pl.multiple_of(i * N, N), N)
                _normalize(xbuf.at[rows], obuf.at[rows], gamma, beta)
                return carry
            lax.fori_loop(lo, hi, body, None)

        def write(lo, hi):
            def body(j, carry):
                for s in range(lo, hi):
                    start = pl.multiple_of(s * N + j * _PIECE, _PIECE)
                    copy(obuf, o_hbm, start, _PIECE, wsem.at[0]).start()
                return carry
            lax.fori_loop(0, N // _PIECE, body, None)

        q = _GROUP
        read_a.wait()
        normalize(0, 2 * q)
        write(0, q)
        write(q, 2 * q)
        normalize(2 * q, n_read)
        read_b.wait()
        normalize(n_read, 3 * q)
        write(2 * q, 3 * q)
        normalize(3 * q, B)
        write(3 * q, B)
        copy(obuf, o_hbm, 0, R, wsem.at[0]).wait()

    xt = x.transpose(0, 2, 3, 1).reshape(R, C)
    y = pl.pallas_call(
        kernel_function,
        in_specs=[pl.BlockSpec(memory_space=pl.ANY)] * 3,
        out_specs=pl.BlockSpec(memory_space=pl.ANY),
        out_shape=jax.ShapeDtypeStruct((R, C), x.dtype),
        scratch_shapes=[
            pltpu.VMEM((R, C), x.dtype),
            pltpu.VMEM((R, C), x.dtype),
            pltpu.VMEM((CT, _LANES), g.dtype),
            pltpu.VMEM((CT, _LANES), b.dtype),
            pltpu.SemaphoreType.DMA((2,)),
            pltpu.SemaphoreType.DMA((1,)),
            pltpu.SemaphoreType.DMA((2,)),
        ],
        compiler_params=pltpu.CompilerParams(vmem_limit_bytes=40 * 1024 * 1024),
    )(xt, g.reshape(CT, _LANES), b.reshape(CT, _LANES))
    return y.reshape(B, H, W, C).transpose(0, 3, 1, 2)
```

```python
import jax
import jax.numpy as jnp
from jax import lax
import jax.experimental.pallas as pl
import jax.experimental.pallas.tpu as pltpu

_EPS = 1e-5
_LANES = 128
_PIECE = 32


def _normalize(x_ref, o_ref, gamma, beta):
    inv_n = 1.0 / x_ref.shape[0]
    xf = x_ref[...].astype(jnp.float32)
    mu = jnp.sum(xf, axis=0, keepdims=True) * inv_n
    d = xf - mu
    var = jnp.sum(d * d, axis=0, keepdims=True) * inv_n
    scale = lax.rsqrt(var + _EPS) * gamma
    o_ref[...] = (d * scale + beta).astype(o_ref.dtype)


@jax.jit
def pallas_standalone__instancenorm__sampling_kernel(
    x: jax.Array,
    g: jax.Array,
    b: jax.Array,
):
    B, C, H, W = x.shape
    N = H * W
    R = B * N
    CT = C // _LANES
    n_w0 = (6 * B) // 16
    n_go = (8 * B) // 16
    n_rd = (10 * B) // 16
    n_w1 = (11 * B) // 16

    def kernel_function(x_hbm, g_hbm, b_hbm, o_hbm,
                        xbuf, obuf, gbuf, bbuf, rsem, wsem, psem):
        def copy(src, dst, start, rows, sem):
            return pltpu.make_async_copy(
                src.at[pl.ds(start, rows)], dst.at[pl.ds(start, rows)], sem)

        read_a = copy(x_hbm, xbuf, 0, n_rd * N, rsem.at[0])
        read_b = copy(x_hbm, xbuf, n_rd * N, R - n_rd * N, rsem.at[1])
        copy_g = pltpu.make_async_copy(g_hbm, gbuf, psem.at[0])
        copy_b = pltpu.make_async_copy(b_hbm, bbuf, psem.at[1])

        read_a.start(priority=1)
        read_b.start(priority=1)
        copy_g.start()
        copy_b.start()
        copy_g.wait()
        copy_b.wait()
        gv = gbuf[...].astype(jnp.float32)
        bv = bbuf[...].astype(jnp.float32)
        gamma = jnp.concatenate([gv[i:i + 1] for i in range(CT)], axis=1)
        beta = jnp.concatenate([bv[i:i + 1] for i in range(CT)], axis=1)

        def normalize(lo, hi):
            def body(i, carry):
                rows = pl.ds(pl.multiple_of(i * N, N), N)
                _normalize(xbuf.at[rows], obuf.at[rows], gamma, beta)
                return carry
            lax.fori_loop(lo, hi, body, None)

        def write(lo, hi):
            def body(j, carry):
                for s in range(lo, hi):
                    start = pl.multiple_of(s * N + j * _PIECE, _PIECE)
                    copy(obuf, o_hbm, start, _PIECE, wsem.at[0]).start()
                return carry
            lax.fori_loop(0, N // _PIECE, body, None)

        read_a.wait()
        normalize(0, n_go)
        write(0, n_w0)
        normalize(n_go, n_rd)
        read_b.wait()
        normalize(n_rd, n_w1)
        write(n_w0, n_w1)
        normalize(n_w1, B)
        write(n_w1, B)
        copy(obuf, o_hbm, 0, R, wsem.at[0]).wait()

    xt = x.transpose(0, 2, 3, 1).reshape(R, C)
    y = pl.pallas_call(
        kernel_function,
        in_specs=[pl.BlockSpec(memory_space=pl.ANY)] * 3,
        out_specs=pl.BlockSpec(memory_space=pl.ANY),
        out_shape=jax.ShapeDtypeStruct((R, C), x.dtype),
        scratch_shapes=[
            pltpu.VMEM((R, C), x.dtype),
            pltpu.VMEM((R, C), x.dtype),
            pltpu.VMEM((CT, _LANES), g.dtype),
            pltpu.VMEM((CT, _LANES), b.dtype),
            pltpu.SemaphoreType.DMA((2,)),
            pltpu.SemaphoreType.DMA((1,)),
            pltpu.SemaphoreType.DMA((2,)),
        ],
        compiler_params=pltpu.CompilerParams(vmem_limit_bytes=40 * 1024 * 1024),
    )(xt, g.reshape(CT, _LANES), b.reshape(CT, _LANES))
    return y.reshape(B, H, W, C).transpose(0, 3, 1, 2)
```
